```python
import os as _os
_os.environ.setdefault("JAX_PLATFORMS", "cpu")
import jax
import jax.numpy as jnp

def _softmax(x, axis=-1):
    return jax.nn.softmax(x, axis=axis)
def _gelu(x):
    return jax.nn.gelu(x, approximate=True)
def _silu(x):
    return jax.nn.silu(x)
def _sigmoid(x):
    return jax.nn.sigmoid(x)
def _layernorm(x, axis=-1, eps=1e-5):
    m = jnp.mean(x, axis=axis, keepdims=True)
    v = jnp.var(x, axis=axis, keepdims=True)
    return (x - m) / jnp.sqrt(v + eps)
def _scatter_add(tgt, idx, src, axis=0):
    return tgt.at[idx].add(src)
def _segment_sum(src, seg, n):
    return jax.ops.segment_sum(src, seg, n)
class _Rng:
    def __init__(self, key):
        self._k = key
    def _next(self):
        self._k, sub = jax.random.split(self._k)
        return sub
    def normal(self, shape):
        return jax.random.normal(self._next(), shape, dtype=jnp.bfloat16)
    def randint(self, lo, hi, shape):
        return jax.random.randint(self._next(), shape, lo, hi, dtype=jnp.int32)
    def uniform(self, shape, lo=0.0, hi=1.0):
        return jax.random.uniform(self._next(), shape, jnp.bfloat16, lo, hi)
    def permutation(self, n):
        return jax.random.permutation(self._next(), n)


kernel_name = 'standalone__gqa_softmax__near_ridge'

def setup_inputs():
    _rng = _Rng(jax.random.key(int.from_bytes(__import__("os").urandom(4), "little")))
    _w = (lambda a: (lambda t: t.astype(jnp.bfloat16) if jnp.issubdtype(t.dtype, jnp.floating) else t)(jnp.asarray(a)))
    B, Hq, Hkv, Sq, Sk, D = 8, 16, 8, 512, 512, 256
    return {
        "q": _w((lambda *s: _rng.normal(s) * 0.4)(B, Hq, Sq, D)),
        "k": _w((lambda *s: _rng.normal(s) * 0.4)(B, Hkv, Sk, D)),
        "v": _w((lambda *s: _rng.normal(s) * 0.05)(B, Hkv, Sk, D)),
    }

def reference(q, k, v):
    B, Hq, Sq, D = q.shape
    Hkv = k.shape[1]
    rep = Hq // Hkv
    k = jnp.repeat(k, rep, axis=1)
    v = jnp.repeat(v, rep, axis=1)
    scale = D ** -0.5
    scores = jnp.einsum("bhqd,bhkd->bhqk", q, k) * scale
    p = _softmax(scores, axis=-1)
    return jnp.einsum("bhqk,bhkd->bhqd", p, v)
```

```python
import math

import jax
import jax.numpy as jnp
from jax import lax
import jax.experimental.pallas as pl
import jax.experimental.pallas.tpu as pltpu


@jax.jit
def pallas_standalone__gqa_softmax__near_ridge_kernel(
    q: jax.Array,
    k: jax.Array,
    v: jax.Array,
):
    B, Hq, Sq, D = q.shape
    Hkv, Sk = k.shape[1], k.shape[2]
    rep = Hq // Hkv
    G = B * Hkv
    M = rep * Sq
    c = (D ** -0.5) * math.log2(math.e)

    def kernel_function(q_ref, k_ref, v_ref, o_ref):
        s = lax.dot_general(
            q_ref[...], k_ref[...], (((1,), (1,)), ((), ())),
            preferred_element_type=jnp.float32)
        m = jnp.max(s, axis=-1, keepdims=True)
        p = jnp.exp2((s - m) * c)
        l = jnp.sum(p, axis=-1, keepdims=True)
        o = jnp.dot(p.astype(v_ref.dtype), v_ref[...],
                    preferred_element_type=jnp.float32)
        o_ref[...] = (o * (1.0 / l)).astype(o_ref.dtype)

    out = pl.pallas_call(
        kernel_function,
        grid=(G,),
        in_specs=[
            pl.BlockSpec((None, M, D), lambda g: (g, 0, 0)),
            pl.BlockSpec((None, Sk, D), lambda g: (g, 0, 0)),
            pl.BlockSpec((None, Sk, D), lambda g: (g, 0, 0)),
        ],
        out_specs=pl.BlockSpec((None, M, D), lambda g: (g, 0, 0)),
        out_shape=jax.ShapeDtypeStruct((G, M, D), q.dtype),
        compiler_params=pltpu.CompilerParams(
            dimension_semantics=("arbitrary",),
            vmem_limit_bytes=64 * 1024 * 1024),
    )(q.reshape(G, M, D), k.reshape(G, Sk, D), v.reshape(G, Sk, D))
    return out.reshape(B, Hq, Sq, D)
```

```python
import math

import jax
import jax.numpy as jnp
from jax import lax
import jax.experimental.pallas as pl
import jax.experimental.pallas.tpu as pltpu

_UNROLL = 16
_SLOTS = 4
_PREFETCH = 2
_TAIL_CHUNKS = 8


@jax.jit
def pallas_standalone__gqa_softmax__near_ridge_kernel(
    q: jax.Array,
    k: jax.Array,
    v: jax.Array,
):
    B, Hq, Sq, D = q.shape
    Hkv, Sk = k.shape[1], k.shape[2]
    rep = Hq // Hkv
    G = B * Hkv
    M = rep * Sq
    assert Hq == rep * Hkv and rep >= 2
    assert q.dtype == k.dtype == v.dtype
    assert G % _UNROLL == 0 and _UNROLL % _SLOTS == 0 and _PREFETCH < _SLOTS
    assert Sq % 32 == 0 and M % (16 * _TAIL_CHUNKS) == 0
    n_iter = G // _UNROLL

    exp2_scale = (D ** -0.5) * math.log2(math.e)

    q_at, k_at, v_at = 0, M, M + Sk
    whole = [(0, M)]
    head_pieces = [(0, Sq // 2), (Sq // 2, Sq // 2), (Sq, M - Sq)]
    tail_rows = M // _TAIL_CHUNKS
    tail_pieces = [(i * tail_rows, tail_rows) for i in range(_TAIL_CHUNKS)]
    kq_sem, v_sem, o_sem, piece_sem = 0, _SLOTS, 2 * _SLOTS, 3 * _SLOTS

    def kernel_function(q_hbm, k_hbm, v_hbm, o_hbm, in_buf, out_buf, sems):
        def load(src, at, g, j, row, rows, sem):
            return pltpu.make_async_copy(
                src.at[g, pl.ds(row, rows)],
                in_buf.at[j % _SLOTS, pl.ds(at + row, rows)],
                sems.at[sem],
            )

        def k_copy(g, j):
            return load(k_hbm, k_at, g, j, 0, Sk, kq_sem + j % _SLOTS)

        def v_copy(g, j):
            return load(v_hbm, v_at, g, j, 0, Sk, v_sem + j % _SLOTS)

        def q_copies(g, j):
            if j % _UNROLL == 0:
                return [
                    load(q_hbm, q_at, g, j, row, rows, piece_sem + i)
                    for i, (row, rows) in enumerate(head_pieces)
                ]
            return [load(q_hbm, q_at, g, j, 0, M, kq_sem + j % _SLOTS)]

        def o_copies(g, j):
            pieces = tail_pieces if j % _UNROLL == _UNROLL - 1 else whole
            return [
                pltpu.make_async_copy(
                    out_buf.at[j % _SLOTS, pl.ds(row, rows)],
                    o_hbm.at[g, pl.ds(row, rows)],
                    sems.at[o_sem + j % _SLOTS],
                )
                for row, rows in pieces
            ]

        def fetch(g, j):
            for copy in [k_copy(g, j), *q_copies(g, j), v_copy(g, j)]:
                copy.start()

        def wait_write_back(g, j):
            for copy in o_copies(g, j):
                copy.wait()

        def q_kt(q_rows, keys):
            return lax.dot_general(
                q_rows,
                keys,
                (((1,), (1,)), ((), ())),
                preferred_element_type=jnp.float32,
            )

        def group(it, j):
            g = it * _UNROLL + j
            slot = j % _SLOTS

            scores = []
            if j == 0:
                k_copy(g, j).wait()
                for copy, (row, rows) in zip(q_copies(g, j), head_pieces):
                    keys = in_buf[slot, pl.ds(k_at, Sk), :]
                    copy.wait()
                    scores.append(
                        q_kt(in_buf[slot, pl.ds(q_at + row, rows), :], keys))
            else:
                for h in range(rep):
                    scores.append(
                        q_kt(in_buf[slot, pl.ds(q_at + h * Sq, Sq), :],
                             in_buf[slot, pl.ds(k_at, Sk), :]))
            s = jnp.concatenate(scores, axis=0)

            if j + _PREFETCH < _UNROLL:
                fetch(g + _PREFETCH, j + _PREFETCH)
            else:
                pl.when(it < n_iter - 1)(
                    lambda: fetch(g + _PREFETCH, j + _PREFETCH))
            if j > 0:
                for copy in o_copies(g - 1, j - 1):
                    copy.start()
            v_copy(g, j).wait()
            if j >= _SLOTS:
                wait_write_back(g - _SLOTS, j - _SLOTS)
            else:
                pl.when(it > 0)(
                    lambda: wait_write_back(g - _SLOTS, j - _SLOTS))

            m = jnp.max(s, axis=-1, keepdims=True)
            p = jnp.exp2((s - m) * exp2_scale).astype(in_buf.dtype)
            l = jnp.sum(p.astype(jnp.float32), axis=-1, keepdims=True)
            inv_l = pltpu.reciprocal(l, approx=True)
            inv_l = inv_l * (2.0 - l * inv_l)
            o = jnp.dot(
                p,
                in_buf[slot, pl.ds(v_at, Sk), :],
                preferred_element_type=jnp.float32,
            )
            o = (o * inv_l).astype(out_buf.dtype)

            if j + 1 < _UNROLL:
                for copy in [k_copy(g + 1, j + 1), *q_copies(g + 1, j + 1)]:
                    copy.wait()
                out_buf[slot] = o
            else:
                for copy, (row, rows) in zip(o_copies(g, j), tail_pieces):
                    out_buf[slot, pl.ds(row, rows), :] = o[row:row + rows]
                    copy.start()

        def iteration(it, carry):
            for j in range(_UNROLL):
                group(it, j)
            return carry

        for g in range(_PREFETCH):
            fetch(g, g)
        lax.fori_loop(0, n_iter, iteration, 0)
        for g in range(G - _SLOTS, G):
            wait_write_back(g, g)

    out = pl.pallas_call(
        kernel_function,
        in_specs=[pl.BlockSpec(memory_space=pl.ANY)] * 3,
        out_specs=pl.BlockSpec(memory_space=pl.ANY),
        out_shape=jax.ShapeDtypeStruct((G, M, D), q.dtype),
        scratch_shapes=[
            pltpu.VMEM((_SLOTS, M + 2 * Sk, D), q.dtype),
            pltpu.VMEM((_SLOTS, M, D), q.dtype),
            pltpu.SemaphoreType.DMA((3 * _SLOTS + len(head_pieces),)),
        ],
        compiler_params=pltpu.CompilerParams(
            vmem_limit_bytes=64 * 1024 * 1024,
            disable_bounds_checks=True,
            flags={"XLA_TPU_RESCHEDULE_DMA_DONES": True},
        ),
    )(q.reshape(G, M, D), k.reshape(G, Sk, D), v.reshape(G, Sk, D))
    return out.reshape(B, Hq, Sq, D)
```
